```python
import os as _os
_os.environ.setdefault("JAX_PLATFORMS", "cpu")
import jax
import jax.numpy as jnp

def _softmax(x, axis=-1):
    return jax.nn.softmax(x, axis=axis)
def _gelu(x):
    return jax.nn.gelu(x, approximate=True)
def _silu(x):
    return jax.nn.silu(x)
def _sigmoid(x):
    return jax.nn.sigmoid(x)
def _layernorm(x, axis=-1, eps=1e-5):
    m = jnp.mean(x, axis=axis, keepdims=True)
    v = jnp.var(x, axis=axis, keepdims=True)
    return (x - m) / jnp.sqrt(v + eps)
def _scatter_add(tgt, idx, src, axis=0):
    return tgt.at[idx].add(src)
def _segment_sum(src, seg, n):
    return jax.ops.segment_sum(src, seg, n)
class _Rng:
    def __init__(self, key):
        self._k = key
    def _next(self):
        self._k, sub = jax.random.split(self._k)
        return sub
    def normal(self, shape):
        return jax.random.normal(self._next(), shape, dtype=jnp.bfloat16)
    def randint(self, lo, hi, shape):
        return jax.random.randint(self._next(), shape, lo, hi, dtype=jnp.int32)
    def uniform(self, shape, lo=0.0, hi=1.0):
        return jax.random.uniform(self._next(), shape, jnp.bfloat16, lo, hi)
    def permutation(self, n):
        return jax.random.permutation(self._next(), n)


kernel_name = 'concat_heads__gqa_block_cached__mha_block_cached__near_ridge'

def setup_inputs():
    _rng = _Rng(jax.random.key(int.from_bytes(__import__("os").urandom(4), "little")))
    _w = (lambda a: (lambda t: t.astype(jnp.bfloat16) if jnp.issubdtype(t.dtype, jnp.floating) else t)(jnp.asarray(a)))
    def _A_setup():
        B, Sq, D = 8, 112, 448
        Hq, Hkv, Sk, Dh = 16, 8, 512, 256
        assert Hq % Hkv == 0, (Hq, Hkv)
        return {
            "x": _w((lambda *s: _rng.normal(s) * 0.8)(B, Sq, D)),
            "k_cache": _w((lambda *s: _rng.normal(s) * 0.8)(B, Hkv, Sk, Dh)),
            "v_cache": _w((lambda *s: _rng.normal(s) * 0.05)(B, Hkv, Sk, Dh)),
            "wq": _w((lambda *s: _rng.normal(s) * 0.8)(D, Hq * Dh) * (D ** -0.5)),
            "wo": _w((lambda *s: _rng.normal(s) * 0.05)(Hq * Dh, D) * ((Hq * Dh) ** -0.5)),
        }
    _A_in = _A_setup()

    def _B_setup():
        B, Sq, D = 8, 112, 448
        H, Sk, Dh = 16, 512, 256
        return {
            "x": _w((lambda *s: _rng.normal(s) * 0.8)(B, Sq, D)),
            "k_cache": _w((lambda *s: _rng.normal(s) * 0.8)(B, H, Sk, Dh)),
            "v_cache": _w((lambda *s: _rng.normal(s) * 0.05)(B, H, Sk, Dh)),
            "wq": _w((lambda *s: _rng.normal(s) * 0.8)(D, H * Dh) * (D ** -0.5)),
            "wo": _w((lambda *s: _rng.normal(s) * 0.05)(H * Dh, D) * ((H * Dh) ** -0.5)),
        }
    _B_in = _B_setup()

    return {
        "A_x": _A_in["x"],
        "A_k_cache": _A_in["k_cache"],
        "A_v_cache": _A_in["v_cache"],
        "A_wq": _A_in["wq"],
        "A_wo": _A_in["wo"],
        "B_x": _B_in["x"],
        "B_k_cache": _B_in["k_cache"],
        "B_v_cache": _B_in["v_cache"],
        "B_wq": _B_in["wq"],
        "B_wo": _B_in["wo"],
    }

def reference(A_x, A_k_cache, A_v_cache, A_wq, A_wo, B_x, B_k_cache, B_v_cache, B_wq, B_wo):
    def _A_ref(x, k_cache, v_cache, wq, wo):
        B, Sq, D = x.shape
        Hq, Dh = 16, 256
        Hkv = k_cache.shape[1]
        rep = Hq // Hkv
        q = (lambda x, *d: x.transpose(*d))((x @ wq).reshape(B, Sq, Hq, Dh), 0, 2, 1, 3)
        k = jnp.repeat(k_cache, rep, axis=1)
        v = jnp.repeat(v_cache, rep, axis=1)
        scores = jnp.einsum("bhqd,bhkd->bhqk", q, k) * (Dh ** -0.5)
        p = _softmax(scores, axis=-1)
        o = jnp.einsum("bhqk,bhkd->bhqd", p, v)
        return (lambda x, *d: x.transpose(*d))(o, 0, 2, 1, 3).reshape(B, Sq, Hq * Dh) @ wo

    def _B_ref(x, k_cache, v_cache, wq, wo):
        B, Sq, D = x.shape
        H, Dh = 16, 256
        q = (lambda x, *d: x.transpose(*d))((x @ wq).reshape(B, Sq, H, Dh), 0, 2, 1, 3)
        scores = jnp.einsum("bhqd,bhkd->bhqk", q, k_cache) * (Dh ** -0.5)
        p = _softmax(scores, axis=-1)
        o = jnp.einsum("bhqk,bhkd->bhqd", p, v_cache)
        return (lambda x, *d: x.transpose(*d))(o, 0, 2, 1, 3).reshape(B, Sq, H * Dh) @ wo

    a = _A_ref(A_x, A_k_cache, A_v_cache, A_wq, A_wo)
    b = _B_ref(B_x, B_k_cache, B_v_cache, B_wq, B_wo)
    return jnp.concatenate([a, b], axis=-1)
```

```python
import functools, math
import jax
import jax.numpy as jnp
import jax.experimental.pallas as pl
import jax.experimental.pallas.tpu as pltpu

B, SQ, D = 8, 112, 448
H, SK, DH = 16, 512, 256
T = B * SQ
NT = T // 128
SCALE = (DH ** -0.5) * math.log2(math.e)
NSLOT = 11
bf16 = jnp.bfloat16
f32 = jnp.float32
NT_DIMS = (((1,), (1,)), ((), ()))

S_XA, S_WQA0, S_WQA8, S_WQA11, S_XB, S_WQB, S_WOA0, S_WOA1, S_WOA4, S_WOB = 0, 1, 5, 6, 7, 8, 9, 10, 11, 12
S_KV = 16
S_FINE = S_KV + 2 * NSLOT
S_OUT = S_FINE + 16
NSEM = S_OUT + NT

A_SEQ = [('qk', 0), ('qk', 1), ('qp', 0, 0), ('dma',), ('pv', 0), ('qk', 2), ('pv', 1), ('qp', 0, 1), ('op', 0),
         ('qk', 3), ('pv', 2), ('qp', 1, 0), ('op', 1), ('qk', 4), ('pv', 3), ('qp', 1, 1), ('op', 2),
         ('qk', 5), ('pv', 4), ('qp', 2, 0), ('op', 3), ('qk', 6), ('pv', 5), ('qk', 7), ('op', 4), ('pv', 6),
         ('pv', 7), ('op', 5), ('qp', 2, 1), ('op', 6)]
B_SEQ = [('qk', 0), ('qk', 1), ('qk', 2), ('dma',), ('pv', 0), ('qk', 3), ('pv', 1), ('qk', 4), ('pv', 2), ('op', 0),
         ('qk', 5), ('pv', 3), ('op', 1), ('qk', 6), ('pv', 4), ('op', 2), ('qk', 7), ('pv', 5), ('op', 3),
         ('pv', 6), ('pv', 7), ('op', 4), ('op', 5), ('op', 6)]
L_SEQ = [('w', 0), ('w', 1), ('w', 2), ('w', 3), ('w', 4),
         ('qk', 0), ('qk', 1), ('qk', 2), ('pv', 0), ('qk', 3), ('pv', 1), ('qk', 4), ('pv', 2), ('op', 0),
         ('pv', 3), ('pv', 4), ('op', 1), ('op', 2), ('op', 3),
         ('w', 5), ('w', 6), ('w', 7),
         ('qk', 5), ('qk', 6), ('qk', 7), ('pv', 5), ('pv', 6), ('pv', 7), ('op', 4), ('op', 5), ('op', 6)]


def otile(os_, j):
    lo = 128 * j - SQ * j
    return jnp.concatenate([os_[j][lo:], os_[j + 1][:128 - (SQ - lo)]], axis=0)


def kernel(xa, ka, va, wqa, wota, xb, kb, vb, wqb, wotb, out_hbm,
           x_v, wq_v, wot_v, q_v, k_v, v_v, acc_v, out_v, sem):

    def cp(src, dst, s):
        return pltpu.make_async_copy(src, dst, sem.at[s])

    def cols(ref, c0, n):
        return ref.at[:, pl.ds(c0, n)]

    c_xa = lambda: cp(xa, x_v.at[0], S_XA)
    c_xb = lambda: cp(xb, x_v.at[1], S_XB)
    c_wqa = lambda i: cp(cols(wqa, i * 512, 512), cols(wq_v.at[0], i * 512, 512), S_WQA0 + i)
    c_wqa8 = lambda: cp(cols(wqa, 8 * DH, 3 * DH), cols(wq_v.at[0], 8 * DH, 3 * DH), S_WQA8)
    c_wqa11 = lambda: cp(cols(wqa, 11 * DH, 5 * DH), cols(wq_v.at[0], 11 * DH, 5 * DH), S_WQA11)
    c_wqb = lambda: cp(wqb, wq_v.at[1], S_WQB)
    c_woa0 = lambda: cp(cols(wota, 0, 512), cols(wot_v.at[0], 0, 512), S_WOA0)
    c_woa1 = lambda: cp(cols(wota, 512, 1536), cols(wot_v.at[0], 512, 1536), S_WOA1)
    c_woa4 = lambda: cp(cols(wota, 2048, 2048), cols(wot_v.at[0], 2048, 2048), S_WOA4)
    c_wob = lambda: cp(wotb, wot_v.at[1], S_WOB)

    def c_kv(kh, vh, h, slot):
        return [cp(kh.at[:, h], k_v.at[slot], S_KV + 2 * slot), cp(vh.at[:, h], v_v.at[slot], S_KV + 2 * slot + 1)]

    LSLOT = (8 + 15) % NSLOT

    def c_fine(b):
        return [cp(kb.at[b, 15], k_v.at[LSLOT, b], S_FINE + 2 * b), cp(vb.at[b, 15], v_v.at[LSLOT, b], S_FINE + 2 * b + 1)]

    def start(cs):
        for c in cs:
            c.start()

    def wait(cs):
        for c in cs:
            c.wait()

    start([c_xa()] + [c_wqa(i) for i in range(4)] + c_kv(ka, va, 0, 0) + [c_woa0(), c_wqa8()]
          + c_kv(ka, va, 1, 1) + [c_wqa11(), c_woa1()])
    acc_v[...] = jnp.zeros(acc_v.shape, f32)
    wait([c_xa()])

    def qproj(br, col, hq, r0, nr, nh=1):
        x = x_v[br, pl.ds(r0, nr), :]
        q = jnp.dot(x, wq_v[br, :, pl.ds(col, nh * DH)], preferred_element_type=f32)
        q = (q * SCALE).astype(bf16)
        for i in range(nh):
            q_v[hq + i, pl.ds(r0, nr), :] = q[:, i * DH:(i + 1) * DH]

    def p_body(i, carry):
        col = pl.multiple_of(i * 512, 512)
        cp(cols(wqa, col, 512), cols(wq_v.at[0], col, 512), S_WQA0 + i).wait()
        for r in range(2):
            for hh in range(2):
                qproj(0, pl.multiple_of(col + hh * DH, DH), 2 * i + hh, r * 448, 448)
        return carry

    jax.lax.fori_loop(0, 4, p_body, 0)

    def softmax(s):
        m = jnp.max(s, axis=-1, keepdims=True)
        p = jnp.exp2(s - m)
        l = jnp.sum(p, axis=-1, keepdims=True)
        return p.astype(bf16), l

    def a_body(g, carry):
        slot = g
        wait(c_kv(ka, va, g, slot))

        @pl.when(g == 0)
        def _():
            wait([c_woa0(), c_wqa8()])

        @pl.when(g == 1)
        def _():
            wait([c_wqa11(), c_woa1()])

        @pl.when(g == 2)
        def _():
            wait([c_xb(), c_wqb()])

        @pl.when(g == 4)
        def _():
            wait([c_woa4()])

        def dma():
            @pl.when(g == 0)
            def _():
                start([c_xb(), c_wqb()])

            @pl.when(g == 1)
            def _():
                start([c_woa4()])

            @pl.when(g == 3)
            def _():
                start([c_wob()])

            @pl.when(g <= 2)
            def _():
                for i in range(2):
                    start(c_kv(ka, va, 2 * g + 2 + i, 2 * g + 2 + i))

            @pl.when(g >= 3)
            def _():
                for i in range(2):
                    pk = 2 * g + 2 + i
                    start(c_kv(kb, vb, pk - 8, pk % NSLOT))

        ss = {}
        os_ = {}
        for item in A_SEQ:
            kind = item[0]
            if kind == 'dma':
                dma()
            elif kind == 'qp':
                hq = 8 + 3 * g + item[1]
                qproj(hq // 16, pl.multiple_of((hq % 16) * DH, DH), hq, item[2] * 448, 448)
            elif kind == 'qk':
                b = item[1]
                q2 = jnp.concatenate([q_v[2 * g, pl.ds(b * SQ, SQ), :], q_v[2 * g + 1, pl.ds(b * SQ, SQ), :]], axis=0)
                ss[b] = jax.lax.dot_general(q2, k_v[slot, b], NT_DIMS, preferred_element_type=f32)
            elif kind == 'pv':
                b = item[1]
                p, l = softmax(ss.pop(b))
                o = jnp.dot(p, v_v[slot, b], preferred_element_type=f32)
                o = (o * pl.reciprocal(l, approx=True)).astype(bf16)
                os_[b] = jnp.concatenate([o[:SQ], o[SQ:]], axis=1)
            elif kind == 'op':
                j = item[1]
                r = jax.lax.dot_general(wot_v[0, :, pl.ds(pl.multiple_of(g * 512, 512), 512)],
                                        otile(os_, j), NT_DIMS, preferred_element_type=f32)
                acc_v[pl.ds(0, D), pl.ds(j * 128, 128)] += r
        return carry

    jax.lax.fori_loop(0, 8, a_body, 0)

    outs = []

    def b_run(h, slot, seq, dma, last):
        ss = {}
        os_ = {}
        col = h * DH if last else pl.multiple_of(h * DH, DH)
        for item in seq:
            kind = item[0]
            if kind == 'dma':
                dma()
            elif kind == 'w':
                wait(c_fine(item[1]))
            elif kind == 'qk':
                b = item[1]
                ss[b] = jax.lax.dot_general(q_v[16 + h, pl.ds(b * SQ, SQ), :], k_v[slot, b], NT_DIMS,
                                            preferred_element_type=f32)
            elif kind == 'pv':
                b = item[1]
                p, l = softmax(ss.pop(b))
                o = jnp.dot(p, v_v[slot, b], preferred_element_type=f32)
                o = (o * pl.reciprocal(l, approx=True)).astype(bf16)
                os_[b] = o
            elif kind == 'op':
                j = item[1]
                ot = otile(os_, j)
                rs = [jax.lax.dot_general(wot_v[1, pl.ds(m * 224, 224), pl.ds(col, DH)], ot, NT_DIMS,
                                          preferred_element_type=f32) for m in range(2)]
                if not last:
                    for m in range(2):
                        acc_v[pl.ds(D + m * 224, 224), pl.ds(j * 128, 128)] += rs[m]
                else:
                    t = jnp.concatenate([acc_v[pl.ds(0, D), pl.ds(j * 128, 128)]] +
                                        [acc_v[pl.ds(D + m * 224, 224), pl.ds(j * 128, 128)] + rs[m] for m in range(2)], axis=0)
                    out_v[pl.ds(j * 128, 128), :] = t.T.astype(bf16)
                    c = cp(out_v.at[pl.ds(j * 128, 128)], out_hbm.at[pl.ds(j * 128, 128)], S_OUT + j)
                    c.start()
                    outs.append(c)

    def b_body(h, carry):
        slot = (8 + h) % NSLOT
        wait(c_kv(kb, vb, h, slot))

        @pl.when(h == 0)
        def _():
            wait([c_wob()])

        def dma():
            nh = h + NSLOT - 1

            @pl.when(nh < 15)
            def _():
                start(c_kv(kb, vb, nh, (8 + nh) % NSLOT))

            @pl.when(nh == 15)
            def _():
                for b in range(B):
                    start(c_fine(b))

        b_run(h, slot, B_SEQ, dma, False)
        return carry

    jax.lax.fori_loop(0, 15, b_body, 0)
    b_run(15, LSLOT, L_SEQ, None, True)
    wait(outs)


@jax.jit
def pallas_concat_heads__gqa_block_cached__mha_block_cached__near_ridge_kernel(
    A_x, A_k_cache, A_v_cache, A_wq, A_wo, B_x, B_k_cache, B_v_cache, B_wq, B_wo):
    hb = pl.BlockSpec(memory_space=pltpu.MemorySpace.HBM)
    out = pl.pallas_call(
        kernel,
        in_specs=[hb] * 10,
        out_specs=hb,
        out_shape=jax.ShapeDtypeStruct((T, 2 * D), bf16),
        scratch_shapes=[
            pltpu.VMEM((2, T, D), bf16),
            pltpu.VMEM((2, D, H * DH), bf16),
            pltpu.VMEM((2, D, H * DH), bf16),
            pltpu.VMEM((2 * H, T, DH), bf16),
            pltpu.VMEM((NSLOT, B, SK, DH), bf16),
            pltpu.VMEM((NSLOT, B, SK, DH), bf16),
            pltpu.VMEM((2 * D, T), f32),
            pltpu.VMEM((T, 2 * D), bf16),
            pltpu.SemaphoreType.DMA((NSEM,)),
        ],
        compiler_params=pltpu.CompilerParams(vmem_limit_bytes=110 * 1024 * 1024, disable_bounds_checks=True),
    )(A_x.reshape(T, D), A_k_cache, A_v_cache, A_wq, A_wo.T,
      B_x.reshape(T, D), B_k_cache, B_v_cache, B_wq, B_wo.T)
    return out.reshape(B, SQ, 2 * D)
```

```python
import math
import jax
import jax.numpy as jnp
import jax.experimental.pallas as pl
import jax.experimental.pallas.tpu as pltpu

B, SQ, D = 8, 112, 448
H, SK, DH = 16, 512, 256
T = B * SQ
NT = T // 128
SCALE = (DH ** -0.5) * math.log2(math.e)
NSLOT = 10
bf16 = jnp.bfloat16
f32 = jnp.float32
NT_DIMS = (((1,), (1,)), ((), ()))

CH = 64
HT = 256
NHT = 16 * 16
P = dict(M0=3, RA=10, XA7=5, RB=21, R6=21, PLOOP=1, DEFER=1)

S_XLO, S_XHI, S_WQ0, S_WQ1, S_WQ2, S_WQN, S_XB, S_WOA, S_WOB, S_WOB7 = range(10)
S_KV = 16
S_FINE = S_KV + 2 * NSLOT
STAGES = {6: [(0, 4), (4, 8)], 7: [(0, 4), (4, 6), (6, 8)]}
FINE = {(i, k): S_FINE + 2 * n for n, (i, k) in enumerate((i, k) for i in (6, 7) for k in range(len(STAGES[i])))}
NSEM = S_FINE + 2 * len(FINE)

A_SEQ = [('qk', 0), ('qk', 1), ('qp', 0, 0), ('pv', 0), ('qk', 2), ('pv', 1), ('qp', 0, 1), ('op', 0),
         ('qk', 3), ('pv', 2), ('qp', 1, 0), ('op', 1), ('qk', 4), ('pv', 3), ('qp', 1, 1), ('op', 2),
         ('qk', 5), ('pv', 4), ('qp', 2, 0), ('op', 3), ('qk', 6), ('pv', 5), ('qk', 7), ('op', 4), ('pv', 6),
         ('pv', 7), ('op', 5), ('qp', 2, 1), ('op', 6)]
COST = {'qk': 1, 'pv': 1, 'op': 1, 'qp': 2}
BCOST = {'qk': 1, 'pv': 1, 'op': 2}


def b_seq(b0, b1, ops, look=2):
    units = [(b, hh) for b in range(b0, b1) for hh in range(2)]
    seq = []
    ops = list(ops)
    for u in range(min(look, len(units))):
        seq.append(('qk',) + units[u])
    done_b = b0 - 1
    for u, (b, hh) in enumerate(units):
        if u + look < len(units):
            seq.append(('qk',) + units[u + look])
        seq.append(('pv', b, hh))
        if ops and ops[0] + 1 <= done_b and u + look < len(units):
            seq.append(('op', ops.pop(0)))
        if hh == 1:
            done_b = b
    seq += [('op', j) for j in ops]
    return seq


def staged_seq(stages):
    seq, j0 = [], 0
    for k, (lo, hi) in enumerate(stages):
        seq += [('w', k)] + b_seq(lo, hi, range(j0, hi - 1))
        j0 = hi - 1
    return seq


def spread(seq, cost, n, skip_first=2, tail=0):
    tot = sum(cost.get(it[0], 0) for it in seq) - tail
    out, acc, k = [], 0, 0
    for idx, it in enumerate(seq):
        out.append(it)
        acc += cost.get(it[0], 0)
        ok = it[0] in ('qk', 'pv') or (it[0] == 'qp' and idx + 1 < len(seq) and seq[idx + 1][0] == 'op')
        while k < n and idx >= skip_first - 1 and (k + 1) * tot <= acc * n + tot // 2 and ok:
            out.append(('ht', k)); k += 1
    assert k == n, (k, n)
    return out


def ht_head(m):
    return ((m >> 5) << 1) + ((m >> 1) & 1)


def otile(os_, j):
    lo = 128 * j - SQ * j
    return jnp.concatenate([os_[j][lo:], os_[j + 1][:128 - (SQ - lo)]], axis=0)


def kernel(xa, ka, va, wqa, wota, xb, kb, vb, wqb, wotb, out_hbm,
           x_v, wq_v, wot_v, q_v, k_v, v_v, acc_v, out_v, sem, osem):
    M0, RA, XA7, RB, R6 = P['M0'], P['RA'], P['XA7'], P['RB'], P['R6']
    X7 = 16 + XA7
    MB0 = M0 + 8 * RA + X7
    M6 = MB0 + 6 * RB
    M7 = min(M6 + R6, NHT)

    assert all(ht_head(m) < 8 for m in range(MB0))
    issued = MB0
    for i in range(6):
        assert issued >= 32 * (i + 1)
        assert all(ht_head(m) - 8 < 2 * i for m in range(issued, issued + RB))
        issued += RB
    assert issued == M6 <= NHT

    def cp(src, dst, s):
        return pltpu.make_async_copy(src, dst, sem.at[s])

    def cols(ref, c0, n):
        return ref.at[:, pl.ds(c0, n)]

    def wait(cs):
        for c in cs:
            c.wait()

    def bslot(head):
        return 2 + (head & 7)

    def chunks(kh, vh, b, head, half, slot, sk):
        for c in range(HT // CH):
            r = half * HT + c * CH
            if not isinstance(r, int):
                r = pl.multiple_of(r, CH)
            cp(kh.at[b, head, pl.ds(r, CH)], k_v.at[slot, b, pl.ds(r, CH)], sk).start(priority=0)
            cp(vh.at[b, head, pl.ds(r, CH)], v_v.at[slot, b, pl.ds(r, CH)], sk + 1).start(priority=1)

    def issue_ht(m, hi):
        assert hi < NHT
        b = (m >> 2) & 7
        pk = m >> 5
        head = ht_head(m)
        slot = bslot(head)
        sk = S_KV + 2 * slot
        for i in (6, 7):
            if isinstance(m, int):
                if pk == i:
                    sk = FINE[i, [k for k, (lo, up) in enumerate(STAGES[i]) if lo <= b < up][0]]
            elif hi >= 32 * i:
                st = sum((b >= lo).astype(jnp.int32) for lo, _ in STAGES[i][1:])
                sk = jnp.where(pk == i, FINE[i, 0] + 2 * st, sk)
        chunks(kb, vb, b, head, m & 1, slot, sk)

    def w_kv(slot):
        return [cp(k_v.at[slot], k_v.at[slot], S_KV + 2 * slot), cp(v_v.at[slot], v_v.at[slot], S_KV + 2 * slot + 1)]

    c_xlo = lambda: cp(xa.at[pl.ds(0, 448)], x_v.at[0, pl.ds(0, 448)], S_XLO)
    c_xhi = lambda: cp(xa.at[pl.ds(448, 448)], x_v.at[0, pl.ds(448, 448)], S_XHI)
    c_wq0 = lambda: cp(cols(wqa, 0, DH), cols(wq_v.at[0], 0, DH), S_WQ0)
    c_wq1 = lambda: cp(cols(wqa, DH, DH), cols(wq_v.at[0], DH, DH), S_WQ1)
    c_wq2 = lambda: cp(cols(wqa, 2 * DH, 6 * DH), cols(wq_v.at[0], 2 * DH, 6 * DH), S_WQ2)
    c_xb = lambda: cp(xb, x_v.at[1], S_XB)
    w_wqn = lambda: cp(cols(wq_v.at[0], 0, 3 * DH), cols(wq_v.at[0], 0, 3 * DH), S_WQN)
    c_woa = lambda g: cp(cols(wota, g * 512, 512), cols(wot_v.at[0], g * 512, 512), S_WOA)
    c_wob = lambda g: cp(cols(wotb, g * 512, 512), cols(wot_v.at[1], g * 512, 512), S_WOB)
    w_wob = lambda: cp(cols(wot_v.at[1], 0, 7 * 512), cols(wot_v.at[1], 0, 7 * 512), S_WOB)
    c_wob7 = lambda: cp(cols(wotb, 7 * 512, 512), cols(wot_v.at[1], 7 * 512, 512), S_WOB7)

    first = [c_xlo(), c_wq0(), c_xhi(), c_wq1(), c_wq2(), c_woa(0)]
    for b in range(B):
        first += [cp(ka.at[b, 0], k_v.at[0, b], S_KV), cp(va.at[b, 0], v_v.at[0, b], S_KV + 1)]
    first += [cp(cols(wqa, 8 * DH, 3 * DH), cols(wq_v.at[0], 8 * DH, 3 * DH), S_WQN), c_xb()]
    for c in first:
        c.start()
    for m in range(M0):
        issue_ht(m, m)
    acc_v[...] = jnp.zeros(acc_v.shape, f32)

    def qproj(br, col, hq, r0, nr):
        x = x_v[br, pl.ds(r0, nr), :]
        q = jnp.dot(x, wq_v[br, :, pl.ds(col, DH)], preferred_element_type=f32)
        q_v[hq, pl.ds(r0, nr), :] = (q * SCALE).astype(bf16)

    wait([c_xlo(), c_wq0()])
    qproj(0, 0, 0, 0, 448)
    wait([c_xhi(), c_wq1()])
    qproj(0, 0, 0, 448, 448)
    qproj(0, DH, 1, 0, 448)
    qproj(0, DH, 1, 448, 448)
    wait([c_wq2()])
    if P['PLOOP']:
        def p_body(it, carry):
            for hh in range(3):
                h = 2 + 3 * it + hh
                for r in range(2):
                    qproj(0, pl.multiple_of(h * DH, DH), h, r * 448, 448)
            return carry
        jax.lax.fori_loop(0, 2, p_body, 0)
    else:
        for h in range(2, 8):
            for r in range(2):
                qproj(0, h * DH, h, r * 448, 448)

    def softmax(s):
        m = jnp.max(s, axis=-1, keepdims=True)
        p = jnp.exp2(s - m)
        l = jnp.sum(p, axis=-1, keepdims=True)
        return p.astype(bf16), l

    a_seq = spread(A_SEQ, COST, 16 + RA, tail=4)

    def a_body(g, carry):
        slot = g & 1
        wait(w_kv(slot) + [w_wqn(), c_woa(g)])

        @pl.when(g == 2)
        def _():
            wait([c_xb()])

        def wdma(i):
            if i < 3:
                hq = 8 + 3 * (g + 1) + i
                col = pl.multiple_of((hq & 15) * DH, DH)

                @pl.when(hq < 16)
                def _():
                    cp(cols(wqa, col, DH), cols(wq_v.at[0], col, DH), S_WQN).start()

                @pl.when(jnp.logical_and(hq >= 16, g < 7))
                def _():
                    cp(cols(wqb, col, DH), cols(wq_v.at[1], col, DH), S_WQN).start()
            elif i == 3:
                @pl.when(g < 7)
                def _():
                    c_woa(g + 1).start()
            else:
                @pl.when(g < 7)
                def _():
                    c_wob(g).start()

        wpos = {2: 0, 5: 1, 8: 2, 11: 3, 14: 4}
        mdyn = M0 + RA * g + jnp.where(g == 7, X7, 0)
        x7 = M0 + RA * 7
        ss = {}
        os_ = {}
        for item in a_seq:
            kind = item[0]
            if kind == 'ht':
                i = item[1]
                if i < 16:
                    pl.when(g < 7)(lambda: chunks(ka, va, i >> 1, g + 1, i & 1, 1 - slot, S_KV + 2 * (1 - slot)))
                    pl.when(g == 7)(lambda: issue_ht(x7, x7))
                    x7 += 1
                    if i in wpos:
                        wdma(wpos[i])
                        if wpos[i] < XA7:
                            pl.when(g == 7)(lambda: issue_ht(x7, x7))
                            x7 += 1
                else:
                    issue_ht(mdyn + (i - 16), MB0 - RA + (i - 16))
            elif kind == 'qp':
                hq = 8 + 3 * g + item[1]
                qproj(hq >> 4, pl.multiple_of((hq & 15) * DH, DH), hq, item[2] * 448, 448)
            elif kind == 'qk':
                b = item[1]
                q2 = jnp.concatenate([q_v[2 * g, pl.ds(b * SQ, SQ), :], q_v[2 * g + 1, pl.ds(b * SQ, SQ), :]], axis=0)
                ss[b] = jax.lax.dot_general(q2, k_v[slot, b], NT_DIMS, preferred_element_type=f32)
            elif kind == 'pv':
                b = item[1]
                p, l = softmax(ss.pop(b))
                o = jnp.dot(p, v_v[slot, b], preferred_element_type=f32)
                o = (o * pl.reciprocal(l, approx=True)).astype(bf16)
                os_[b] = jnp.concatenate([o[:SQ], o[SQ:]], axis=1)
            elif kind == 'op':
                j = item[1]
                r = jax.lax.dot_general(wot_v[0, :, pl.ds(pl.multiple_of(g * 512, 512), 512)],
                                        otile(os_, j), NT_DIMS, preferred_element_type=f32)
                acc_v[pl.ds(0, D), pl.ds(j * 128, 128)] += r
        assert x7 == M0 + RA * 7 + X7
        return carry

    jax.lax.fori_loop(0, 8, a_body, 0)

    outs = []

    def emit_out(j, r):
        bpart = acc_v[pl.ds(D, D), pl.ds(j * 128, 128)]
        if r is not None:
            bpart = bpart + r
        t = jnp.concatenate([acc_v[pl.ds(0, D), pl.ds(j * 128, 128)], bpart], axis=0)
        out_v[pl.ds(j * 128, 128), :] = t.T.astype(bf16)
        c = pltpu.make_async_copy(out_v.at[pl.ds(j * 128, 128)], out_hbm.at[pl.ds(j * 128, 128)], osem.at[j])
        c.start()
        outs.append(c)

    def b_run(i, seq, m0, mhi):
        static = isinstance(i, int)
        last = static and i == 7
        ss, oh, os_ = {}, {}, {}
        slots = [bslot(2 * i), bslot(2 * i + 1)]
        col = i * 512 if static else pl.multiple_of(i * 512, 512)
        deferred = []
        nht = 0
        for n, item in enumerate(seq):
            kind = item[0]
            if kind == 'ht':
                k = item[1]
                issue_ht(m0 + k, mhi + k)
                nht += 1
            elif kind == 'wob7':
                c_wob7().start()
            elif kind == 'w':
                lo, hi = STAGES[i][item[1]]
                assert m0 + nht >= 32 * i + 4 * hi
                kw = k_v.at[pl.ds(slots[0], 2), pl.ds(lo, hi - lo)]
                vw = v_v.at[pl.ds(slots[0], 2), pl.ds(lo, hi - lo)]
                wait([cp(kw, kw, FINE[i, item[1]]), cp(vw, vw, FINE[i, item[1]] + 1)])
                if last and item[1] == 0:
                    wait([c_wob7()])
                for j in deferred:
                    emit_out(j, None)
                deferred = []
            elif kind == 'qk':
                _, b, hh = item
                ss[b, hh] = jax.lax.dot_general(q_v[16 + 2 * i + hh, pl.ds(b * SQ, SQ), :], k_v[slots[hh], b], NT_DIMS,
                                                preferred_element_type=f32)
            elif kind == 'pv':
                _, b, hh = item
                p, l = softmax(ss.pop((b, hh)))
                o = jnp.dot(p, v_v[slots[hh], b], preferred_element_type=f32)
                oh[b, hh] = (o * pl.reciprocal(l, approx=True)).astype(bf16)
                if hh == 1:
                    os_[b] = jnp.concatenate([oh.pop((b, 0)), oh.pop((b, 1))], axis=1)
            elif kind == 'op':
                j = item[1]
                r = jax.lax.dot_general(wot_v[1, :, pl.ds(col, 512)], otile(os_, j), NT_DIMS,
                                        preferred_element_type=f32)
                stage_end = n + 1 < len(seq) and seq[n + 1][0] == 'w'
                if last and not (P['DEFER'] and stage_end):
                    emit_out(j, r)
                else:
                    acc_v[pl.ds(D, D), pl.ds(j * 128, 128)] += r
                    if last:
                        deferred.append(j)

    b_sq = spread(b_seq(0, 8, range(7)), BCOST, RB, tail=4)

    def b_body(i, carry):
        wait(w_kv(bslot(2 * i)) + w_kv(bslot(2 * i + 1)))

        @pl.when(i == 0)
        def _():
            wait([w_wob()])

        b_run(i, b_sq, MB0 + RB * i, MB0 + RB * 5)
        return carry

    jax.lax.fori_loop(0, 6, b_body, 0)

    assert all(ht_head(m) - 8 < 12 for m in range(M6, NHT))
    s6 = spread(staged_seq(STAGES[6]), BCOST, M7 - M6, skip_first=3, tail=4)
    k6 = max(32 * 7 - M6, 1) - 1
    p6 = s6.index(('ht', min(k6, M7 - M6 - 1)))
    s6 = s6[:p6 + 1] + [('wob7',)] + s6[p6 + 1:]
    b_run(6, s6, M6, M6)
    s7 = staged_seq(STAGES[7])
    w1 = s7.index(('w', 1))
    if NHT > M7:
        s7 = spread(s7[:w1], BCOST, NHT - M7, skip_first=3, tail=4) + s7[w1:]
    b_run(7, s7, M7, M7)
    wait(outs)


@jax.jit
def pallas_concat_heads__gqa_block_cached__mha_block_cached__near_ridge_kernel(
    A_x, A_k_cache, A_v_cache, A_wq, A_wo, B_x, B_k_cache, B_v_cache, B_wq, B_wo):
    hb = pl.BlockSpec(memory_space=pltpu.MemorySpace.HBM)
    out = pl.pallas_call(
        kernel,
        in_specs=[hb] * 10,
        out_specs=hb,
        out_shape=jax.ShapeDtypeStruct((T, 2 * D), bf16),
        scratch_shapes=[
            pltpu.VMEM((2, T, D), bf16),
            pltpu.VMEM((2, D, H * DH), bf16),
            pltpu.VMEM((2, D, H * DH), bf16),
            pltpu.VMEM((2 * H, T, DH), bf16),
            pltpu.VMEM((NSLOT, B, SK, DH), bf16),
            pltpu.VMEM((NSLOT, B, SK, DH), bf16),
            pltpu.VMEM((2 * D, T), f32),
            pltpu.VMEM((T, 2 * D), bf16),
            pltpu.SemaphoreType.DMA((NSEM,)),
            pltpu.SemaphoreType.DMA((NT,)),
        ],
        compiler_params=pltpu.CompilerParams(vmem_limit_bytes=110 * 1024 * 1024, disable_bounds_checks=True,
                                             disable_semaphore_checks=True),
    )(A_x.reshape(T, D), A_k_cache, A_v_cache, A_wq, A_wo.T,
      B_x.reshape(T, D), B_k_cache, B_v_cache, B_wq, B_wo.T)
    return out.reshape(B, SQ, 2 * D)
```

```python
import math

import jax
import jax.numpy as jnp
import jax.experimental.pallas as pl
import jax.experimental.pallas.tpu as pltpu

B, SQ, D = 8, 112, 448
H, SK, DH = 16, 512, 256
T = B * SQ
NT = T // 128
SCALE = (DH ** -0.5) * math.log2(math.e)
bf16 = jnp.bfloat16
f32 = jnp.float32
NT_DIMS = (((1,), (1,)), ((), ()))

NSLOT = 10
CH = 64
HT = 256
NHT = 16 * 16
NLOOP = 6
MT = 32 * NLOOP
AW = 384

M0 = 3
RA = 10
G0 = 2
X7 = 16 + 5
RB = 21
TSTEP = 2.0
TB = (0, 6, 10, 13, 15, 16)
MB0 = M0 + 8 * RA + X7 - G0
ML = MB0 + NLOOP * RB

S_XLO, S_XHI, S_WQ0, S_WQ1, S_WQ2, S_WA, S_XB, S_WOB, S_WOB7 = range(9)
S_KVA = 9
S_KVB = 11
S_TAIL = 15
NSEM = S_TAIL + len(TB) - 1

A_SEQ = [('qk', 0), ('qk', 1), ('qp', 0, 0), ('pv', 0), ('qk', 2), ('pv', 1), ('qp', 0, 1), ('op', 0),
         ('qk', 3), ('pv', 2), ('qp', 1, 0), ('op', 1), ('qk', 4), ('pv', 3), ('qp', 1, 1), ('op', 2),
         ('qk', 5), ('pv', 4), ('qp', 2, 0), ('op', 3), ('qk', 6), ('pv', 5), ('qk', 7), ('op', 4), ('pv', 6),
         ('pv', 7), ('op', 5), ('qp', 2, 1), ('op', 6)]
A_COST = {'qk': 1, 'pv': 1, 'op': 1, 'qp': 2}
B_COST = {'qk': 1, 'pv': 1, 'op': 2}


def _b_seq(c0, c1, ops, look=2):
    units = [(c, hh) for c in range(c0, c1) for hh in range(2)]
    seq = [('qk',) + u for u in units[:look]]
    done = c0 - 1
    for u, (c, hh) in enumerate(units):
        if u + look < len(units):
            seq.append(('qk',) + units[u + look])
        seq.append(('pv', c, hh))
        if ops and ops[0] + 1 <= done and u + look < len(units):
            seq.append(('op', ops.pop(0)))
        if hh == 1:
            done = c
    while ops and ops[0] + 1 <= done:
        seq.append(('op', ops.pop(0)))
    return seq


def _spread(seq, cost, n, step, skip_first=2):
    out, acc, k = [], 0, 0
    for idx, it in enumerate(seq):
        out.append(it)
        acc += cost.get(it[0], 0)
        ok = it[0] in ('qk', 'pv') or (it[0] == 'qp' and idx + 1 < len(seq) and seq[idx + 1][0] == 'op')
        while k < n and idx >= skip_first - 1 and (k + 0.5) * step <= acc and ok:
            out.append(('ht', k))
            k += 1
    assert k == n, (k, n)
    return out


def _ht_head(m):
    return ((m >> 5) << 1) + ((m >> 1) & 1)


def _check_plan():
    assert all(_ht_head(m) < 8 for m in range(MB0)) and G0 <= 7
    for i in range(NLOOP):
        assert MB0 + RB * i >= 32 * (i + 1)
        assert all(_ht_head(m) - 8 < 2 * i for m in range(MB0 + RB * i, MB0 + RB * (i + 1)))
    assert ML <= NHT and all(_ht_head(m) - 8 < 2 * NLOOP for m in range(ML, NHT))


def _otile(os_, c):
    lo = (128 - SQ) * (c % B)
    return jnp.concatenate([os_[c][lo:], os_[c + 1][:128 - (SQ - lo)]], axis=0)


def _softmax(s):
    m = jnp.max(s, axis=-1, keepdims=True)
    p = jnp.exp2(s - m)
    l = jnp.sum(p, axis=-1, keepdims=True)
    return p.astype(bf16), pl.reciprocal(l, approx=True)


def _kernel(xa, ka, va, wqa, wota, xb, kb, vb, wqb, wotb, out_hbm,
            x_v, wq_v, wot_v, q_v, k_v, v_v, acc_v, out_v, sem, osem):
    _check_plan()

    def cp(src, dst, s):
        return pltpu.make_async_copy(src, dst, sem.at[s])

    def wait(cs):
        for c in cs:
            c.wait()

    def aligned(x, n):
        return x if isinstance(x, int) else pl.multiple_of(x, n)

    def bslot(head):
        return 2 + (head & 7)

    def chunks(kh, vh, b, head, half, slot, sm):
        for c in range(HT // CH):
            r = aligned(half * HT + c * CH, CH)
            cp(kh.at[b, head, pl.ds(r, CH)], k_v.at[slot, b, pl.ds(r, CH)], sm).start(priority=0)
            cp(vh.at[b, head, pl.ds(r, CH)], v_v.at[slot, b, pl.ds(r, CH)], sm).start(priority=1)

    def issue_ht(m, hi):
        assert hi < NHT
        head = _ht_head(m)
        sm = S_KVB + ((m >> 5) & 3)
        if isinstance(m, int):
            if m >= MT:
                sm = S_TAIL + sum(m >= MT + 4 * t for t in TB[1:-1])
        elif hi >= MT:
            st = sum((m >= MT + 4 * t).astype(jnp.int32) for t in TB[1:-1] if hi >= MT + 4 * t)
            sm = jnp.where(m >= MT, S_TAIL + st, sm)
        chunks(kb, vb, (m >> 2) & 7, head, m & 1, bslot(head), sm)

    def w_tiles(n, nb, sm):
        r = k_v.at[pl.ds(0, n), pl.ds(0, nb)]
        return cp(r, r, sm)

    def c_wq(src, hq, sm):
        return cp(src.at[:, pl.ds(aligned((hq & 15) * DH, DH), DH)], wq_v.at[hq], sm)

    def c_wo(src, g, dst, sm):
        return cp(src.at[:, pl.ds(aligned(g * 512, 512), 512)], wot_v.at[dst], sm)

    c_xlo = lambda: cp(xa.at[pl.ds(0, 448)], x_v.at[0, pl.ds(0, 448)], S_XLO)
    c_xhi = lambda: cp(xa.at[pl.ds(448, 448)], x_v.at[0, pl.ds(448, 448)], S_XHI)
    c_xb = lambda: cp(xb, x_v.at[1], S_XB)
    c_wob7 = lambda: c_wo(wotb, 7, 15, S_WOB7)
    w_wq2 = lambda: cp(wq_v.at[pl.ds(2, 6)], wq_v.at[pl.ds(2, 6)], S_WQ2)
    w_wa = lambda: cp(wq_v.at[pl.ds(0, 5)], wq_v.at[pl.ds(0, 5)], S_WA)
    w_wob = lambda: cp(wot_v.at[pl.ds(8, 7)], wot_v.at[pl.ds(8, 7)], S_WOB)

    first = [c_xlo(), c_wq(wqa, 0, S_WQ0), c_xhi(), c_wq(wqa, 1, S_WQ1)]
    first += [c_wq(wqa, h, S_WQ2) for h in range(2, 8)] + [c_wo(wota, 0, 0, S_WA)]
    for b in range(B):
        first += [cp(ka.at[b, 0], k_v.at[0, b], S_KVA), cp(va.at[b, 0], v_v.at[0, b], S_KVA)]
    first += [c_wq(wqa, h, S_WA) for h in range(8, 11)] + [c_xb()]
    for c in first:
        c.start()
    for m in range(M0):
        issue_ht(m, m)
    acc_v[...] = jnp.zeros(acc_v.shape, f32)

    def qproj(br, hq, r0):
        q = jnp.dot(x_v[br, pl.ds(r0, 448), :], wq_v[hq], preferred_element_type=f32)
        q_v[hq, pl.ds(r0, 448), :] = (q * SCALE).astype(bf16)

    wait([c_xlo(), c_wq(wqa, 0, S_WQ0)])
    qproj(0, 0, 0)
    wait([c_xhi(), c_wq(wqa, 1, S_WQ1)])
    qproj(0, 0, 448)
    qproj(0, 1, 0)
    qproj(0, 1, 448)
    wait([w_wq2()])
    for h in range(2, 8):
        for r in range(2):
            qproj(0, h, r * 448)

    a_seq = _spread(A_SEQ, A_COST, 16 + RA, (sum(A_COST[i[0]] for i in A_SEQ) - 4) / (16 + RA))

    def a_body(g, carry):
        slot = g & 1
        wait([w_tiles(2, B, S_KVA + slot), w_wa()])

        @pl.when(g == 2)
        def _():
            wait([c_xb()])

        def wdma(i):
            if i < 3:
                hq = 8 + 3 * (g + 1) + i

                @pl.when(hq < 16)
                def _():
                    c_wq(wqa, hq, S_WA).start()

                @pl.when(jnp.logical_and(hq >= 16, g < 7))
                def _():
                    c_wq(wqb, hq, S_WA).start()
            elif i == 3:
                @pl.when(g < 7)
                def _():
                    c_wo(wota, g + 1, g + 1, S_WA).start()
            else:
                @pl.when(g < 7)
                def _():
                    c_wo(wotb, g, 8 + g, S_WOB).start()

        wpos = {2: 0, 5: 1, 8: 2, 11: 3, 14: 4}
        mdyn = M0 + RA * g - jnp.minimum(g, G0) + jnp.where(g == 7, X7, 0)
        x7 = M0 + RA * 7 - G0
        ss = {}
        os_ = {}
        for item in a_seq:
            kind = item[0]
            if kind == 'ht':
                i = item[1]
                if i < 16:
                    pl.when(g < 7)(lambda: chunks(ka, va, i >> 1, g + 1, i & 1, 1 - slot, S_KVA + 1 - slot))
                    pl.when(g == 7)(lambda: issue_ht(x7, x7))
                    x7 += 1
                    if i in wpos:
                        wdma(wpos[i])
                        pl.when(g == 7)(lambda: issue_ht(x7, x7))
                        x7 += 1
                elif i == 16 + RA - 1:
                    pl.when(g >= G0)(lambda: issue_ht(mdyn + (i - 16), MB0 - RA + (i - 16)))
                else:
                    issue_ht(mdyn + (i - 16), MB0 - RA + (i - 16))
            elif kind == 'qp':
                hq = 8 + 3 * g + item[1]
                qproj(hq >> 4, hq, item[2] * 448)
            elif kind == 'qk':
                b = item[1]
                q2 = jnp.concatenate([q_v[2 * g, pl.ds(b * SQ, SQ), :], q_v[2 * g + 1, pl.ds(b * SQ, SQ), :]],
                                     axis=0)
                ss[b] = jax.lax.dot_general(q2, k_v[slot, b], NT_DIMS, preferred_element_type=f32)
            elif kind == 'pv':
                b = item[1]
                p, rl = _softmax(ss.pop(b))
                o = (jnp.dot(p, v_v[slot, b], preferred_element_type=f32) * rl).astype(bf16)
                os_[b] = jnp.concatenate([o[:SQ], o[SQ:]], axis=1)
            else:
                j = item[1]
                r = jax.lax.dot_general(wot_v[g], _otile(os_, j), NT_DIMS, preferred_element_type=f32)
                acc_v[pl.ds(0, D), pl.ds(j * 128, 128)] += r
        assert x7 == M0 + RA * 7 - G0 + X7
        return carry

    jax.lax.fori_loop(0, 8, a_body, 0)

    outs = []
    pend = []

    def out_copy(rows, c0, n, s):
        return pltpu.make_async_copy(out_v.at[rows, pl.ds(c0, n)], out_hbm.at[rows, pl.ds(c0, n)], osem.at[s])

    def flush_out():
        for c in pend:
            c.start(priority=1)
            outs.append(c)
        pend.clear()

    def emit_out(j, r, hold):
        bpart = acc_v[pl.ds(D, D), pl.ds(j * 128, 128)]
        if r is not None:
            bpart = bpart + r
        t = jnp.concatenate([acc_v[pl.ds(AW, D - AW), pl.ds(j * 128, 128)], bpart], axis=0)
        out_v[pl.ds(j * 128, 128), pl.ds(AW, 2 * D - AW)] = t.T.astype(bf16)
        pend.append(out_copy(pl.ds(j * 128, 128), AW, 2 * D - AW, j))
        if not hold:
            flush_out()

    def b_run(i0, seq, m0, mhi, tail):
        ss, oh, os_ = {}, {}, {}
        deferred = []
        nht = 0
        hold = True
        for n, item in enumerate(seq):
            kind = item[0]
            if kind == 'ht':
                issue_ht(m0 + item[1], mhi + item[1])
                nht += 1
                if tail and nht == max(MT + 32 - m0, 1):
                    c_wob7().start()
            elif kind == 'w':
                k = item[1]
                assert m0 + nht >= MT + 4 * TB[k + 1]
                wait([w_tiles(4, TB[k + 1] - TB[k], S_TAIL + k)])
                if TB[k] <= B < TB[k + 1]:
                    assert nht >= max(MT + 32 - m0, 1)
                    wait([c_wob7()])
                if k == 0:
                    for j in range(NT):
                        out_v[pl.ds(j * 128, 128), pl.ds(0, AW)] = (
                            acc_v[pl.ds(0, AW), pl.ds(j * 128, 128)].T.astype(bf16))
                    pend.append(out_copy(pl.ds(0, T), 0, AW, NT))
                if k == len(TB) - 3:
                    hold = False
                    flush_out()
                for j in deferred:
                    emit_out(j, None, hold)
                deferred = []
            elif kind == 'qk':
                _, c, hh = item
                head = 2 * (i0 + c // B) + hh
                ss[c, hh] = jax.lax.dot_general(q_v[16 + head, pl.ds((c % B) * SQ, SQ), :],
                                                k_v[bslot(head), c % B], NT_DIMS, preferred_element_type=f32)
            elif kind == 'pv':
                _, c, hh = item
                head = 2 * (i0 + c // B) + hh
                p, rl = _softmax(ss.pop((c, hh)))
                oh[c, hh] = (jnp.dot(p, v_v[bslot(head), c % B], preferred_element_type=f32) * rl).astype(bf16)
                if hh == 1:
                    os_[c] = jnp.concatenate([oh.pop((c, 0)), oh.pop((c, 1))], axis=1)
            else:
                c = item[1]
                j = c % B
                r = jax.lax.dot_general(wot_v[8 + i0 + c // B], _otile(os_, c), NT_DIMS,
                                        preferred_element_type=f32)
                final = tail and c >= B
                if final and not (n + 1 < len(seq) and seq[n + 1][0] == 'w'):
                    emit_out(j, r, hold)
                else:
                    acc_v[pl.ds(D, D), pl.ds(j * 128, 128)] += r
                    if final:
                        deferred.append(j)

    b_sq = _b_seq(0, B, list(range(NT)))
    b_sq = _spread(b_sq, B_COST, RB, (sum(B_COST[i[0]] for i in b_sq) - 4) / RB)

    def b_body(i, carry):
        wait([w_tiles(4, B, S_KVB + (i & 3))])

        @pl.when(i == 0)
        def _():
            wait([w_wob()])

        b_run(i, b_sq, MB0 + RB * i, MB0 + RB * (NLOOP - 1), False)
        return carry

    jax.lax.fori_loop(0, NLOOP, b_body, 0)

    ops = list(range(NT)) + list(range(B, B + NT))
    t_sq = []
    for k in range(len(TB) - 1):
        t_sq += [('w', k)] + _b_seq(TB[k], TB[k + 1], ops)
    assert not ops
    b_run(NLOOP, _spread(t_sq, B_COST, NHT - ML, TSTEP, skip_first=3), ML, ML, True)
    assert not pend and len(outs) == NT + 1
    wait(outs)


@jax.jit
def pallas_concat_heads__gqa_block_cached__mha_block_cached__near_ridge_kernel(
    A_x: jax.Array,
    A_k_cache: jax.Array,
    A_v_cache: jax.Array,
    A_wq: jax.Array,
    A_wo: jax.Array,
    B_x: jax.Array,
    B_k_cache: jax.Array,
    B_v_cache: jax.Array,
    B_wq: jax.Array,
    B_wo: jax.Array,
):
    hbm = pl.BlockSpec(memory_space=pltpu.MemorySpace.HBM)
    out = pl.pallas_call(
        _kernel,
        in_specs=[hbm] * 10,
        out_specs=hbm,
        out_shape=jax.ShapeDtypeStruct((T, 2 * D), bf16),
        scratch_shapes=[
            pltpu.VMEM((2, T, D), bf16),
            pltpu.VMEM((2 * H, D, DH), bf16),
            pltpu.VMEM((H, D, 512), bf16),
            pltpu.VMEM((2 * H, T, DH), bf16),
            pltpu.VMEM((NSLOT, B, SK, DH), bf16),
            pltpu.VMEM((NSLOT, B, SK, DH), bf16),
            pltpu.VMEM((2 * D, T), f32),
            pltpu.VMEM((T, 2 * D), bf16),
            pltpu.SemaphoreType.DMA((NSEM,)),
            pltpu.SemaphoreType.DMA((NT + 1,)),
        ],
        compiler_params=pltpu.CompilerParams(vmem_limit_bytes=110 * 1024 * 1024, disable_bounds_checks=True,
                                             disable_semaphore_checks=True),
    )(A_x.reshape(T, D), A_k_cache, A_v_cache, A_wq, A_wo.T,
      B_x.reshape(T, D), B_k_cache, B_v_cache, B_wq, B_wo.T)
    return out.reshape(B, SQ, 2 * D)
```
